```python
import jax
import jax.numpy as jnp

def _softmax(x, axis=-1):
    return jax.nn.softmax(x, axis=axis)
def _gelu(x):
    return jax.nn.gelu(x, approximate=True)
def _silu(x):
    return jax.nn.silu(x)
def _sigmoid(x):
    return jax.nn.sigmoid(x)
def _layernorm(x, axis=-1, eps=1e-5):
    m = jnp.mean(x, axis=axis, keepdims=True)
    v = jnp.var(x, axis=axis, keepdims=True)
    return (x - m) / jnp.sqrt(v + eps)
def _scatter_add(tgt, idx, src, axis=0):
    return tgt.at[idx].add(src)
def _segment_sum(src, seg, n):
    return jax.ops.segment_sum(src, seg, n)
class _Rng:
    def __init__(self, key):
        self._k = key
    def _next(self):
        self._k, sub = jax.random.split(self._k)
        return sub
    def normal(self, shape):
        return jax.random.normal(self._next(), shape, dtype=jnp.bfloat16)
    def randint(self, lo, hi, shape):
        return jax.random.randint(self._next(), shape, lo, hi, dtype=jnp.int32)
    def uniform(self, shape, lo=0.0, hi=1.0):
        return jax.random.uniform(self._next(), shape, jnp.bfloat16, lo, hi)
    def permutation(self, n):
        return jax.random.permutation(self._next(), n)


kernel_name = 'interleave_layers__sliding_local_dilated__mixer_token_mlp__prompt'

def setup_inputs():
    _rng = _Rng(jax.random.key(int.from_bytes(__import__("os").urandom(4), "little")))
    _w = (lambda a: (lambda t: t.astype(jnp.bfloat16) if jnp.issubdtype(t.dtype, jnp.floating) else t)(jnp.asarray(a)))
    def _A_setup():
        B, S, D = 1, 2048, 1024
        return {
            "x": _w((lambda *s: _rng.normal(s) * 0.05)(B, S, D)),
            "wqkv": _w((lambda *s: _rng.normal(s) * 0.05)(D, 3 * D)),
            "wo": _w((lambda *s: _rng.normal(s) * 0.05)(D, D)),
        }
    _A_in = _A_setup()

    def _B_setup():
        B, S, D, F = 1, 2048, 1024, 3584
        return {
            "x": _w((lambda *s: _rng.normal(s) * 0.05)(B, S, D)),
            "w1": _w((lambda *s: _rng.normal(s) * 0.05)(S, F) * (S ** -0.5)),
            "b1": _w((lambda *s: _rng.normal(s) * 0.05)(F) * 0.02),
            "w2": _w((lambda *s: _rng.normal(s) * 0.05)(F, S) * (F ** -0.5)),
            "b2": _w((lambda *s: _rng.normal(s) * 0.05)(S) * 0.02),
        }
    _B_in = _B_setup()

    return {
        "A_x": _A_in["x"],
        "A_wqkv": _A_in["wqkv"],
        "A_wo": _A_in["wo"],
        "B_x": _B_in["x"],
        "B_w1": _B_in["w1"],
        "B_b1": _B_in["b1"],
        "B_w2": _B_in["w2"],
        "B_b2": _B_in["b2"],
    }

def reference(A_x, A_wqkv, A_wo, B_x, B_w1, B_b1, B_w2, B_b2):
    def _A_ref(x, wqkv, wo):
        B, S, D = x.shape
        H = 32; Dh = D // H
        W, dil = 8, 2
        qkv = (lambda x, *d: x.transpose(*d))((x @ wqkv).reshape(B, S, 3, H, Dh), 2, 0, 3, 1, 4)
        q, k, v = qkv[0], qkv[1], qkv[2]
        scale = Dh ** -0.5
        pos = jnp.arange(S)
        off = jnp.arange(W) * dil
        idx = pos[:, None] - off[None, :]
        mask = idx >= 0
        idx_c = jnp.where(mask, idx, 0).reshape(-1)
        kg = k[:, :, idx_c, :].reshape(B, H, S, W, Dh)
        vg = v[:, :, idx_c, :].reshape(B, H, S, W, Dh)
        logits = jnp.einsum("bhsd,bhswd->bhsw", q, kg) * scale
        logits = jnp.where(mask[None, None, :, :], logits, -1e9)
        attn = _softmax(logits, axis=-1)
        o = jnp.einsum("bhsw,bhswd->bhsd", attn, vg)
        return (lambda x, *d: x.transpose(*d))(o, 0, 2, 1, 3).reshape(B, S, D) @ wo

    def _B_ref(x, w1, b1, w2, b2):
        B, S, D = x.shape
        h = _layernorm(x, axis=-1)
        u = jnp.einsum("bsd,sf->bdf", h, w1) + b1
        u = _gelu(u)
        y = jnp.einsum("bdf,fs->bds", u, w2) + b2
        return (lambda x, *d: x.transpose(*d))(y, 0, 2, 1)

    x = A_x
    x = x + _A_ref(_layernorm(x, axis=-1), A_wqkv, A_wo)
    x = x + _B_ref(_layernorm(x, axis=-1), B_w1, B_b1, B_w2, B_b2)
    x = x + _A_ref(_layernorm(x, axis=-1), A_wqkv, A_wo)
    x = x + _B_ref(_layernorm(x, axis=-1), B_w1, B_b1, B_w2, B_b2)
    return x
```

```python
import math

import jax
import jax.numpy as jnp
import jax.experimental.pallas as pl
import jax.experimental.pallas.tpu as pltpu

S, D, F = 2048, 1024, 3584
H, DH, W, DIL = 32, 32, 8, 2
EPS = 1e-5
T = 256
NT = S // T
FC = 512
NF = F // FC
TB = 512
NB = S // TB
HALO = 16
NJ = D // 128
f32, bf16 = jnp.float32, jnp.bfloat16


def _dot(a, b):
    return jnp.dot(a, b, preferred_element_type=f32)


def _dot_nt(a, b):
    return jax.lax.dot_general(a, b, (((1,), (1,)), ((), ())), preferred_element_type=f32)


def _center(x):
    m = jnp.sum(x, axis=-1, keepdims=True) * (1.0 / D)
    c = x - m
    v = jnp.sum(c * c, axis=-1, keepdims=True) * (1.0 / D)
    return c, v


def _ln(x):
    c, v = _center(x)
    return c * jax.lax.rsqrt(v + EPS)


def _ln_ln(x):
    c, v = _center(x)
    r = jax.lax.rsqrt(v + EPS)
    return c * (r * jax.lax.rsqrt(v * r * r + EPS))


def _gelu(x):
    k = math.sqrt(2.0 / math.pi)
    hx = 0.5 * x
    return hx + hx * jnp.tanh(x * (k + (k * 0.044715) * (x * x)))


def _kernel(x_hbm, wqkv_hbm, wo_hbm, w1_hbm, b1_ref, w2_hbm, b2_ref, out_hbm,
            xio, wraw, woraw, wt, wo, w1, w2, xs, ha, ht, u, tmp,
            qn, kn, vn, qc, kc, vc, oc, sem_in, sem_w1, sem_w2, sem_out):
    cp_w = [pltpu.make_async_copy(wqkv_hbm.at[:, pl.ds(s * D, D)], wraw.at[s], sem_in.at[s]) for s in range(3)]
    cp_x = pltpu.make_async_copy(x_hbm, xio, sem_in.at[3])
    cp_wo = pltpu.make_async_copy(wo_hbm, woraw, sem_in.at[4])
    cp_w1 = [pltpu.make_async_copy(w1_hbm.at[:, pl.ds(i * FC, FC)], w1.at[i], sem_w1.at[i]) for i in range(NF)]
    cp_w2 = [pltpu.make_async_copy(w2_hbm.at[:, pl.ds(i * TB, TB)], w2.at[i], sem_w2.at[i]) for i in range(NB)]
    for c in cp_w + [cp_x, cp_wo] + cp_w1 + cp_w2:
        c.start()

    def permute_rows_from_tmp(store):
        for d in range(DH):
            store(d, tmp[pl.ds(d, H, stride=DH), :].astype(bf16))

    for s in range(3):
        cp_w[s].wait()

        def body(kt, _, s=s):
            r0 = pl.multiple_of(kt * 128, 128)
            tmp[...] = wraw[s, pl.ds(r0, 128), :].astype(f32).T

            def st(d, val):
                wt[s, pl.ds(d * H, H), pl.ds(r0, 128)] = val
            permute_rows_from_tmp(st)
        jax.lax.fori_loop(0, D // 128, body, None)

    cp_x.wait()

    def ln0(i, _):
        r0 = pl.multiple_of(i * 128, 128)
        x = xio[pl.ds(r0, 128), :].astype(f32)
        xs[pl.ds(r0, 128), :] = x
        ha[pl.ds(r0, 128), :] = _ln(x).astype(bf16)
    jax.lax.fori_loop(0, S // 128, ln0, None)

    cp_wo.wait()
    for j in range(NJ):
        tmp[...] = woraw[:, pl.ds(j * 128, 128)].astype(f32)

        def st(d, val, j=j):
            wo[pl.ds(d * H, H), pl.ds(j * 128, 128)] = val
        permute_rows_from_tmp(st)

    def proj(r0, s, dst):
        y = _dot_nt(ha[pl.ds(r0, T), :], wt[s])
        for j in range(NJ):
            dst[j] = y[:, j * 128:(j + 1) * 128]

    def advance():
        for j in range(NJ):
            kc[j, pl.ds(0, HALO), :] = kc[j, pl.ds(T, HALO), :]
            vc[j, pl.ds(0, HALO), :] = vc[j, pl.ds(T, HALO), :]
        for j in range(NJ):
            qc[j] = qn[j]
            kc[j, pl.ds(HALO, T), :] = kn[j]
            vc[j, pl.ds(HALO, T), :] = vn[j]

    cexp = (DH ** -0.5) * math.log2(math.e)
    neg = -1e9 / (DH ** -0.5)

    def attend8(r0, r):
        q = [qc[j, pl.ds(r, 8), :] for j in range(NJ)]
        lg = []
        for w in range(W):
            o = HALO + r - DIL * w
            a = q[0] * kc[0, pl.ds(o, 8), :]
            for j in range(1, NJ):
                a = a + q[j] * kc[j, pl.ds(o, 8), :]
            a = a + pltpu.roll(a, 64, 1)
            a = a + pltpu.roll(a, 32, 1)
            if r < DIL * w:
                pos = r0 + r + jax.lax.broadcasted_iota(jnp.int32, (8, 128), 0)
                a = jnp.where(pos >= DIL * w, a, neg)
            lg.append(a)
        m = lg[0]
        for w in range(1, W):
            m = jnp.maximum(m, lg[w])
        e = [jnp.exp2((l - m) * cexp) for l in lg]
        z = e[0]
        for w in range(1, W):
            z = z + e[w]
        inv = 1.0 / z
        p = [x * inv for x in e]
        out = []
        for j in range(NJ):
            a = p[0] * vc[j, pl.ds(HALO + r, 8), :]
            for w in range(1, W):
                a = a + p[w] * vc[j, pl.ds(HALO + r - DIL * w, 8), :]
            out.append(a)
        return out

    def attend(r0):
        for r in range(0, T, 16):
            a, b = attend8(r0, r), attend8(r0, r + 8)
            for j in range(NJ):
                oc[pl.ds(r, 16), pl.ds(j * 128, 128)] = jnp.concatenate([a[j], b[j]], axis=0).astype(bf16)

    def out_proj(r0):
        x = xs[pl.ds(r0, T), :] + _dot(oc[...], wo[...])
        xs[pl.ds(r0, T), :] = x
        return x

    def mix_in(r0, x):
        ht[:, pl.ds(r0, T)] = _ln_ln(x).T.astype(bf16)

    def layer(l, _):
        for j in range(NJ):
            z = jnp.zeros((HALO, 128), f32)
            kc[j, pl.ds(T, HALO), :] = z
            vc[j, pl.ds(T, HALO), :] = z
        proj(0, 0, qn)
        proj(0, 1, kn)
        proj(0, 2, vn)

        def a_body(i, _):
            r0 = pl.multiple_of(i * T, T)
            rp = pl.multiple_of(r0 - T, T)
            advance()
            proj(r0, 0, qn)
            attend(rp)
            proj(r0, 1, kn)
            x = out_proj(rp)
            proj(r0, 2, vn)
            mix_in(rp, x)
        jax.lax.fori_loop(1, NT, a_body, None)
        advance()
        attend(S - T)
        mix_in(S - T, out_proj(S - T))

        @pl.when(l == 0)
        def _():
            for c in cp_w1 + cp_w2:
                c.wait()

        def b1_body(i, _):
            c0 = pl.multiple_of(i * FC, FC)
            u[:, pl.ds(c0, FC)] = _gelu(_dot(ht[...], w1[i]) + b1_ref[i]).astype(bf16)
        jax.lax.fori_loop(0, NF, b1_body, None)

        def b2_body(i, _):
            yt = _dot(u[...], w2[i]) + b2_ref[i]
            for t in range(TB // 128):
                r0 = pl.multiple_of(i * TB + t * 128, 128)
                x = xs[pl.ds(r0, 128), :] + yt[:, t * 128:(t + 1) * 128].T
                xs[pl.ds(r0, 128), :] = x
                xio[pl.ds(r0, 128), :] = x.astype(bf16)
                ha[pl.ds(r0, 128), :] = _ln(x).astype(bf16)

            @pl.when(l == 1)
            def _():
                r0 = pl.multiple_of(i * TB, TB)
                pltpu.make_async_copy(xio.at[pl.ds(r0, TB)], out_hbm.at[pl.ds(r0, TB)], sem_out.at[i]).start()
        jax.lax.fori_loop(0, NB, b2_body, None)

    jax.lax.fori_loop(0, 2, layer, None)
    for i in range(NB):
        pltpu.make_async_copy(xio.at[pl.ds(i * TB, TB)], out_hbm.at[pl.ds(i * TB, TB)], sem_out.at[i]).wait()


@jax.jit
def pallas_interleave_layers__sliding_local_dilated__mixer_token_mlp__prompt_kernel(
    A_x, A_wqkv, A_wo, B_x, B_w1, B_b1, B_w2, B_b2,
):
    del B_x
    any_spec = pl.BlockSpec(memory_space=pl.ANY)
    vmem_spec = pl.BlockSpec(memory_space=pltpu.VMEM)
    out = pl.pallas_call(
        _kernel,
        out_shape=jax.ShapeDtypeStruct((S, D), bf16),
        in_specs=[any_spec, any_spec, any_spec, any_spec, vmem_spec, any_spec, vmem_spec],
        out_specs=any_spec,
        scratch_shapes=[
            pltpu.VMEM((S, D), bf16),
            pltpu.VMEM((3, D, D), bf16),
            pltpu.VMEM((D, D), bf16),
            pltpu.VMEM((3, D, D), bf16),
            pltpu.VMEM((D, D), bf16),
            pltpu.VMEM((NF, S, FC), bf16),
            pltpu.VMEM((NB, F, TB), bf16),
            pltpu.VMEM((S, D), f32),
            pltpu.VMEM((S, D), bf16),
            pltpu.VMEM((D, S), bf16),
            pltpu.VMEM((D, F), bf16),
            pltpu.VMEM((D, 128), f32),
            pltpu.VMEM((NJ, T, 128), f32),
            pltpu.VMEM((NJ, T, 128), f32),
            pltpu.VMEM((NJ, T, 128), f32),
            pltpu.VMEM((NJ, T, 128), f32),
            pltpu.VMEM((NJ, T + HALO, 128), f32),
            pltpu.VMEM((NJ, T + HALO, 128), f32),
            pltpu.VMEM((T, D), bf16),
            pltpu.SemaphoreType.DMA((5,)),
            pltpu.SemaphoreType.DMA((NF,)),
            pltpu.SemaphoreType.DMA((NB,)),
            pltpu.SemaphoreType.DMA((NB,)),
        ],
        compiler_params=pltpu.CompilerParams(vmem_limit_bytes=110 * 1024 * 1024),
        name="interleave_layers",
    )(A_x.reshape(S, D), A_wqkv, A_wo, B_w1, B_b1.reshape(NF, 1, FC), B_w2, B_b2.reshape(NB, 1, TB))
    return out.reshape(1, S, D)
```

```python
import math

import jax
import jax.numpy as jnp
import jax.experimental.pallas as pl
import jax.experimental.pallas.tpu as pltpu

S, D, F = 2048, 1024, 3584
H, DH, W, DIL = 32, 32, 8, 2
EPS = 1e-5
T = 256
NT = S // T
FC = 512
NF = F // FC
TB = 512
NB = S // TB
HALO = 16
NJ = D // 128
f32, bf16 = jnp.float32, jnp.bfloat16


def _dot(a, b):
    return jnp.dot(a, b, preferred_element_type=f32)


def _dot_nt(a, b):
    return jax.lax.dot_general(a, b, (((1,), (1,)), ((), ())), preferred_element_type=f32)


def _center(x):
    m = jnp.sum(x, axis=-1, keepdims=True) * (1.0 / D)
    c = x - m
    v = jnp.sum(c * c, axis=-1, keepdims=True) * (1.0 / D)
    return c, v


def _ln(x):
    c, v = _center(x)
    return c * jax.lax.rsqrt(v + EPS)


def _ln_ln(x):
    c, v = _center(x)
    r = jax.lax.rsqrt(v + EPS)
    return c * (r * jax.lax.rsqrt(v * r * r + EPS))


def _gelu(x):
    k = math.sqrt(2.0 / math.pi)
    hx = 0.5 * x
    return hx + hx * jnp.tanh(x * (k + (k * 0.044715) * (x * x)))


def _kernel(x_hbm, wqkv_hbm, wo_hbm, w1_hbm, b1_ref, w2_hbm, b2_ref, out_hbm,
            xio, wraw, woraw, wt, wo, w1, w2, xs, ha, ht, u,
            qn, kn, vn, qc, kc, vc, oc, sem_in, sem_w1, sem_w2, sem_out):
    cp_w = [pltpu.make_async_copy(wqkv_hbm.at[:, pl.ds(s * D, D)], wraw.at[s], sem_in.at[s]) for s in range(3)]
    cp_x = pltpu.make_async_copy(x_hbm, xio, sem_in.at[3])
    cp_wo = pltpu.make_async_copy(wo_hbm, woraw, sem_in.at[4])
    cp_w1 = [pltpu.make_async_copy(w1_hbm.at[:, pl.ds(i * FC, FC)], w1.at[i], sem_w1.at[i]) for i in range(NF)]
    cp_w2 = [pltpu.make_async_copy(w2_hbm.at[:, pl.ds(i * TB, TB)], w2.at[i], sem_w2.at[i]) for i in range(NB)]
    cp_w[0].start()
    cp_x.start()

    def permute_rows(y):
        sub = jax.lax.broadcasted_iota(jnp.int32, (8, 128), 0)
        res = {}
        for g in range(H // 8):
            for dq in range(DH // 8):
                v = [y[(8 * g + i) * DH + 8 * dq:(8 * g + i) * DH + 8 * dq + 8] for i in range(8)]
                for st in (4, 2, 1):
                    lo = (sub & st) == 0
                    for i in range(8):
                        if i & st == 0:
                            p, q = v[i], v[i + st]
                            v[i] = jnp.where(lo, p, pltpu.roll(q, st, 0))
                            v[i + st] = jnp.where(lo, pltpu.roll(p, 8 - st, 0), q)
                for i in range(8):
                    res[8 * dq + i, g] = v[i]
        return jnp.concatenate([res[d, g] for d in range(DH) for g in range(H // 8)], axis=0).astype(bf16)

    def prep_w(s):
        for kt in range(NJ):
            wt[s, :, pl.ds(kt * 128, 128)] = permute_rows(wraw[s, pl.ds(kt * 128, 128), :].astype(f32).T)

    def ln0(lo, hi):
        for r0 in range(lo, hi, 128):
            x = xio[pl.ds(r0, 128), :].astype(f32)
            xs[pl.ds(r0, 128), :] = x
            ha[pl.ds(r0, 128), :] = _ln(x).astype(bf16)

    def proj(r0, s, dst):
        y = _dot_nt(ha[pl.ds(r0, T), :], wt[s])
        for j in range(NJ):
            dst[j] = y[:, j * 128:(j + 1) * 128]

    def advance():
        for j in range(NJ):
            kc[j, pl.ds(0, HALO), :] = kc[j, pl.ds(T, HALO), :]
            vc[j, pl.ds(0, HALO), :] = vc[j, pl.ds(T, HALO), :]
        for j in range(NJ):
            qc[j] = qn[j]
            kc[j, pl.ds(HALO, T), :] = kn[j]
            vc[j, pl.ds(HALO, T), :] = vn[j]

    cexp = (DH ** -0.5) * math.log2(math.e)
    neg = -1e9 / (DH ** -0.5)

    def attend8(r0, r):
        q = [qc[j, pl.ds(r, 8), :] for j in range(NJ)]
        lg = []
        for w in range(W):
            o = HALO + r - DIL * w
            a = q[0] * kc[0, pl.ds(o, 8), :]
            for j in range(1, NJ):
                a = a + q[j] * kc[j, pl.ds(o, 8), :]
            a = a + pltpu.roll(a, 64, 1)
            a = a + pltpu.roll(a, 32, 1)
            if r < DIL * w:
                pos = r0 + r + jax.lax.broadcasted_iota(jnp.int32, (8, 128), 0)
                a = jnp.where(pos >= DIL * w, a, neg)
            lg.append(a)
        m = lg[0]
        for w in range(1, W):
            m = jnp.maximum(m, lg[w])
        e = [jnp.exp2((l - m) * cexp) for l in lg]
        z = e[0]
        for w in range(1, W):
            z = z + e[w]
        inv = 1.0 / z
        p = [x * inv for x in e]
        out = []
        for j in range(NJ):
            a = p[0] * vc[j, pl.ds(HALO + r, 8), :]
            for w in range(1, W):
                a = a + p[w] * vc[j, pl.ds(HALO + r - DIL * w, 8), :]
            out.append(a)
        return out

    def projt(r0, s, j, dep=None):
        h = ha[pl.ds(r0, T), :]
        if dep is not None: h = jnp.concatenate([jnp.where(r0 < 0, dep.astype(f32), h[:16].astype(f32)).astype(bf16), h[16:]], axis=0)
        y = _dot_nt(h, wt[s, pl.ds(j * 128, 128*1), :])
        for a in range(1): (qn, kn, vn)[s][j+a] = y[:, a*128:a*128+128]

    def attend(r0, rows=range(0, T, 16)):
        for r in rows:
            a, b = attend8(r0, r), attend8(r0, r + 8)
            for j in range(NJ):
                oc[pl.ds(r, 16), pl.ds(j * 128, 128)] = jnp.concatenate([a[j], b[j]], axis=0).astype(bf16)
        return jnp.concatenate([jnp.concatenate([a[j], b[j]], axis=0) for j in range(NJ)], axis=1)

    def out_proj(r0):
        x = xs[pl.ds(r0, T), :] + _dot(oc[...], wo[...])
        xs[pl.ds(r0, T), :] = x
        return x

    def mix_in(r0, x):
        ht[:, pl.ds(r0, T)] = _ln_ln(x).T.astype(bf16)

    def layer(l, _):
        for j in range(NJ):
            z = jnp.zeros((HALO, 128), f32)
            kc[j, pl.ds(T, HALO), :] = z
            vc[j, pl.ds(T, HALO), :] = z

        def a_body(i, _):
            r0 = pl.multiple_of(i * T, T)
            rp = pl.multiple_of(r0 - T, T)
            advance()
            dep = None
            for n in range(0,2 * NJ,1):
                projt(r0, n // NJ, n % NJ, dep)
                dep = attend(rp,range(16*n,16*(n+1),16))
            x = out_proj(rp)
            dep, hs = None, []
            for j in range(NJ):
                projt(r0, 2, j, dep)
                if j < 4:
                    hs.append(_ln_ln(x[64 * j:64 * j + 64]))
                    dep = hs[j][48:]
                elif j < 6:
                    t = (j - 4) * 128
                    hh = jnp.concatenate(hs[2 * (j - 4):2 * (j - 3)], axis=0).T.astype(bf16)
                    ht[:, pl.ds(pl.multiple_of(rp + t, 128), 128)] = hh
                    dep = jnp.concatenate([hh[128 * a + 112:128 * a + 128] for a in range(NJ)], axis=1)
                else:
                    dep = None
        jax.lax.fori_loop(1, NT, a_body, None)
        advance()
        attend(S - T)
        mix_in(S - T, out_proj(S - T))

        @pl.when(l == 0)
        def _():
            for c in cp_w1 + cp_w2:
                c.wait()

        def b1_body(i, _):
            c0 = pl.multiple_of(i * FC, FC)
            u[:, pl.ds(c0, FC)] = _gelu(_dot(ht[...], w1[i]) + b1_ref[:, pl.ds(c0, FC)]).astype(bf16)
        jax.lax.fori_loop(0, NF, b1_body, None)

        def b2_body(i, _):
            yt = _dot(u[...], w2[i]) + b2_ref[:, pl.ds(pl.multiple_of(i * TB, TB), TB)]
            for t in range(TB // 128):
                r0 = pl.multiple_of(i * TB + t * 128, 128)
                x = xs[pl.ds(r0, 128), :] + yt[:, t * 128:(t + 1) * 128].T
                xs[pl.ds(r0, 128), :] = x
                xio[pl.ds(r0, 128), :] = x.astype(bf16)
                ha[pl.ds(r0, 128), :] = _ln(x).astype(bf16)

            @pl.when(l == 1)
            def _():
                r0 = pl.multiple_of(i * TB, TB)
                pltpu.make_async_copy(xio.at[pl.ds(r0, TB)], out_hbm.at[pl.ds(r0, TB)], sem_out.at[i]).start()
        jax.lax.fori_loop(0, NB, b2_body, None)

        @pl.when(l == 0)
        def _():
            proj(0, 0, qn)
            proj(0, 1, kn)
            proj(0, 2, vn)

    cp_w[0].wait()
    for c in cp_w[1:] + [cp_wo]:
        c.start()
    prep_w(0)
    cp_x.wait()
    cp_w[1].wait()
    for c in cp_w1 + cp_w2:
        c.start()
    ln0(0, T)
    proj(0, 0, qn)
    prep_w(1)
    ln0(T, 4 * T)
    cp_w[2].wait()
    proj(0, 1, kn)
    prep_w(2)
    ln0(4 * T, 6 * T)
    cp_wo.wait()
    proj(0, 2, vn)
    ln0(6 * T, S)
    for j in range(NJ):
        wo[:, pl.ds(j * 128, 128)] = permute_rows(woraw[:, pl.ds(j * 128, 128)].astype(f32))
    jax.lax.fori_loop(0, 2, layer, None)
    for i in range(NB):
        pltpu.make_async_copy(xio.at[pl.ds(i * TB, TB)], out_hbm.at[pl.ds(i * TB, TB)], sem_out.at[i]).wait()


@jax.jit
def pallas_interleave_layers__sliding_local_dilated__mixer_token_mlp__prompt_kernel(
    A_x, A_wqkv, A_wo, B_x, B_w1, B_b1, B_w2, B_b2,
):
    del B_x
    any_spec = pl.BlockSpec(memory_space=pl.ANY)
    vmem_spec = pl.BlockSpec(memory_space=pltpu.VMEM)
    out = pl.pallas_call(
        _kernel,
        out_shape=jax.ShapeDtypeStruct((S, D), bf16),
        in_specs=[any_spec, any_spec, any_spec, any_spec, vmem_spec, any_spec, vmem_spec],
        out_specs=any_spec,
        scratch_shapes=[
            pltpu.VMEM((S, D), bf16),
            pltpu.VMEM((3, D, D), bf16),
            pltpu.VMEM((D, D), bf16),
            pltpu.VMEM((3, D, D), bf16),
            pltpu.VMEM((D, D), bf16),
            pltpu.VMEM((NF, S, FC), bf16),
            pltpu.VMEM((NB, F, TB), bf16),
            pltpu.VMEM((S, D), f32),
            pltpu.VMEM((S, D), bf16),
            pltpu.VMEM((D, S), bf16),
            pltpu.VMEM((D, F), bf16),
            pltpu.VMEM((NJ, T, 128), f32),
            pltpu.VMEM((NJ, T, 128), f32),
            pltpu.VMEM((NJ, T, 128), f32),
            pltpu.VMEM((NJ, T, 128), f32),
            pltpu.VMEM((NJ, T + HALO, 128), f32),
            pltpu.VMEM((NJ, T + HALO, 128), f32),
            pltpu.VMEM((T, D), bf16),
            pltpu.SemaphoreType.DMA((5,)),
            pltpu.SemaphoreType.DMA((NF,)),
            pltpu.SemaphoreType.DMA((NB,)),
            pltpu.SemaphoreType.DMA((NB,)),
        ],
        compiler_params=pltpu.CompilerParams(vmem_limit_bytes=110 * 1024 * 1024),
        name="interleave_layers",
    )(A_x.reshape(S, D), A_wqkv, A_wo, B_w1, B_b1.reshape(1, F), B_w2, B_b2.reshape(1, S))
    return out.reshape(1, S, D)
```

```python
import math

import jax
import jax.numpy as jnp
import jax.experimental.pallas as pl
import jax.experimental.pallas.tpu as pltpu

S, D, F = 2048, 1024, 3584
H, DH, W, DIL = 32, 32, 8, 2
EPS = 1e-5
T = 256
NT = S // T
FC = 512
NF = F // FC
TB = 512
NB = S // TB
HALO = 16
NJ = D // 128
f32, bf16 = jnp.float32, jnp.bfloat16


def _dot(a, b):
    return jnp.dot(a, b, preferred_element_type=f32)


def _dot_nt(a, b):
    return jax.lax.dot_general(a, b, (((1,), (1,)), ((), ())), preferred_element_type=f32)


def _center(x):
    m = jnp.sum(x, axis=-1, keepdims=True) * (1.0 / D)
    c = x - m
    v = jnp.sum(c * c, axis=-1, keepdims=True) * (1.0 / D)
    return c, v


def _ln(x):
    c, v = _center(x)
    return c * jax.lax.rsqrt(v + EPS)


def _ln_ln(x):
    c, v = _center(x)
    r = jax.lax.rsqrt(v + EPS)
    return c * (r * jax.lax.rsqrt(v * r * r + EPS))


def _gelu(x):
    k = math.sqrt(2.0 / math.pi)
    hx = 0.5 * x
    return hx + hx * jnp.tanh(x * (k + (k * 0.044715) * (x * x)))


def _kernel(x_hbm, wqkv_hbm, wo_hbm, w1_hbm, b1_ref, w2_hbm, b2_ref, out_hbm,
            xio, wraw, woraw, wt, wo, w1, w2, xs, ha, ht, u,
            qn, kn, vn, qc, kc, vc, oc, sem_in, sem_w1, sem_w2, sem_out):
    cp_w = [pltpu.make_async_copy(wqkv_hbm.at[:, pl.ds(s * D, D)], wraw.at[s], sem_in.at[s]) for s in range(3)]
    cp_x = pltpu.make_async_copy(x_hbm.at[pl.ds(0, T)], xio.at[pl.ds(0, T)], sem_in.at[3])
    cp_x2 = pltpu.make_async_copy(x_hbm.at[pl.ds(T, S - T)], xio.at[pl.ds(T, S - T)], sem_in.at[5])
    cp_wo = pltpu.make_async_copy(wo_hbm, woraw, sem_in.at[4])
    cp_w1 = [pltpu.make_async_copy(w1_hbm.at[:, pl.ds(i * FC, FC)], w1.at[i], sem_w1.at[i]) for i in range(NF)]
    cp_w2 = [pltpu.make_async_copy(w2_hbm.at[:, pl.ds(i * TB, TB)], w2.at[i], sem_w2.at[i]) for i in range(NB)]
    cp_w[0].start()
    cp_x.start()

    def permute_rows(y):
        sub = jax.lax.broadcasted_iota(jnp.int32, (8, 128), 0)
        res = {}
        for g in range(H // 8):
            for dq in range(DH // 8):
                v = [y[(8 * g + i) * DH + 8 * dq:(8 * g + i) * DH + 8 * dq + 8] for i in range(8)]
                for st in (4, 2, 1):
                    lo = (sub & st) == 0
                    for i in range(8):
                        if i & st == 0:
                            p, q = v[i], v[i + st]
                            v[i] = jnp.where(lo, p, pltpu.roll(q, st, 0))
                            v[i + st] = jnp.where(lo, pltpu.roll(p, 8 - st, 0), q)
                for i in range(8):
                    res[8 * dq + i, g] = v[i]
        return jnp.concatenate([res[d, g] for d in range(DH) for g in range(H // 8)], axis=0).astype(bf16)

    def prep_w(s):
        for kt in range(NJ):
            wt[s, :, pl.ds(kt * 128, 128)] = permute_rows(wraw[s, pl.ds(kt * 128, 128), :].astype(f32).T)

    def ln0(lo, hi):
        for r0 in range(lo, hi, 128):
            x = xio[pl.ds(r0, 128), :].astype(f32)
            xs[pl.ds(r0, 128), :] = x
            ha[pl.ds(r0, 128), :] = _ln(x).astype(bf16)

    def proj(r0, s, dst):
        y = _dot_nt(ha[pl.ds(r0, T), :], wt[s])
        for j in range(NJ):
            dst[j] = y[:, j * 128:(j + 1) * 128]

    def advance():
        for j in range(NJ):
            kc[j, pl.ds(0, HALO), :] = kc[j, pl.ds(T, HALO), :]
            vc[j, pl.ds(0, HALO), :] = vc[j, pl.ds(T, HALO), :]
        for j in range(NJ):
            qc[j] = qn[j]
            kc[j, pl.ds(HALO, T), :] = kn[j]
            vc[j, pl.ds(HALO, T), :] = vn[j]

    cexp = (DH ** -0.5) * math.log2(math.e)
    neg = -1e9 / (DH ** -0.5)

    def attend8(r0, r):
        q = [qc[j, pl.ds(r, 8), :] for j in range(NJ)]
        lg = []
        for w in range(W):
            o = HALO + r - DIL * w
            a = q[0] * kc[0, pl.ds(o, 8), :]
            for j in range(1, NJ):
                a = a + q[j] * kc[j, pl.ds(o, 8), :]
            a = a + pltpu.roll(a, 64, 1)
            a = a + pltpu.roll(a, 32, 1)
            if r < DIL * w:
                pos = r0 + r + jax.lax.broadcasted_iota(jnp.int32, (8, 128), 0)
                a = jnp.where(pos >= DIL * w, a, neg)
            lg.append(a)
        m = lg[0]
        for w in range(1, W):
            m = jnp.maximum(m, lg[w])
        e = [jnp.exp2((l - m) * cexp) for l in lg]
        z = e[0]
        for w in range(1, W):
            z = z + e[w]
        inv = 1.0 / z
        p = [x * inv for x in e]
        out = []
        for j in range(NJ):
            a = p[0] * vc[j, pl.ds(HALO + r, 8), :]
            for w in range(1, W):
                a = a + p[w] * vc[j, pl.ds(HALO + r - DIL * w, 8), :]
            out.append(a)
        return out

    def projt(r0, s, j, dep=None):
        h = ha[pl.ds(r0, T), :]
        if dep is not None: h = jnp.concatenate([jnp.where(r0 < 0, dep.astype(f32), h[:16].astype(f32)).astype(bf16), h[16:]], axis=0)
        y = _dot_nt(h, wt[s, pl.ds(j * 128, 128*1), :])
        for a in range(1): (qn, kn, vn)[s][j+a] = y[:, a*128:a*128+128]

    def attend(r0, rows=range(0, T, 16)):
        for r in rows:
            a, b = attend8(r0, r), attend8(r0, r + 8)
            for j in range(NJ):
                oc[pl.ds(r, 16), pl.ds(j * 128, 128)] = jnp.concatenate([a[j], b[j]], axis=0).astype(bf16)
        return jnp.concatenate([jnp.concatenate([a[j], b[j]], axis=0) for j in range(NJ)], axis=1)

    def out_proj(r0):
        x = xs[pl.ds(r0, T), :] + _dot(oc[...], wo[...])
        xs[pl.ds(r0, T), :] = x
        return x

    def mix_in(r0, x):
        ht[:, pl.ds(r0, T)] = _ln_ln(x).T.astype(bf16)

    def layer(l, _):
        for j in range(NJ):
            z = jnp.zeros((HALO, 128), f32)
            kc[j, pl.ds(T, HALO), :] = z
            vc[j, pl.ds(T, HALO), :] = z

        def a_body(i, _):
            r0 = pl.multiple_of(i * T, T)
            rp = pl.multiple_of(r0 - T, T)
            advance()
            dep = None
            for n in range(0,2 * NJ,1):
                projt(r0, n // NJ, n % NJ, dep)
                dep = attend(rp,range(16*n,16*(n+1),16))
            x = out_proj(rp)
            dep, hs = None, []
            for j in range(NJ):
                projt(r0, 2, j, dep)
                if j < 4:
                    hs.append(_ln_ln(x[64 * j:64 * j + 64]))
                    dep = hs[j][48:]
                elif j < 6:
                    t = (j - 4) * 128
                    hh = jnp.concatenate(hs[2 * (j - 4):2 * (j - 3)], axis=0).T.astype(bf16)
                    ht[:, pl.ds(pl.multiple_of(rp + t, 128), 128)] = hh
                    dep = jnp.concatenate([hh[128 * a + 112:128 * a + 128] for a in range(NJ)], axis=1)
                else:
                    dep = None
        jax.lax.fori_loop(1, NT, a_body, None)
        advance()
        attend(S - T)
        mix_in(S - T, out_proj(S - T))

        @pl.when(l == 0)
        def _():
            for c in cp_w1 + cp_w2:
                c.wait()

        def b1_body(i, _):
            c0 = pl.multiple_of(i * FC, FC)
            u[:, pl.ds(c0, FC)] = _gelu(_dot(ht[...], w1[i]) + b1_ref[pl.ds(c0, FC)].astype(f32).reshape(1, FC)).astype(bf16)
        jax.lax.fori_loop(0, NF, b1_body, None)

        def b2_body(i, _):
            yt = _dot(u[...], w2[i]) + b2_ref[pl.ds(pl.multiple_of(i * TB, TB), TB)].astype(f32).reshape(1, TB)
            for t in range(TB // 128):
                r0 = pl.multiple_of(i * TB + t * 128, 128)
                x = xs[pl.ds(r0, 128), :] + yt[:, t * 128:(t + 1) * 128].T
                xs[pl.ds(r0, 128), :] = x
                xio[pl.ds(r0, 128), :] = x.astype(bf16)
                ha[pl.ds(r0, 128), :] = _ln(x).astype(bf16)

            @pl.when(l == 1)
            def _():
                r0 = pl.multiple_of(i * TB, TB)
                pltpu.make_async_copy(xio.at[pl.ds(r0, TB)], out_hbm.at[pl.ds(r0, TB)], sem_out.at[i]).start()
        jax.lax.fori_loop(0, NB, b2_body, None)

        @pl.when(l == 0)
        def _():
            proj(0, 0, qn)
            proj(0, 1, kn)
            proj(0, 2, vn)

    cp_w[0].wait()
    cp_x.wait()
    cp_w[1].start()
    prep_w(0)
    ln0(0, T)
    cp_w[1].wait()
    cp_w[2].start()
    proj(0, 0, qn)
    prep_w(1)
    cp_w[2].wait()
    cp_x2.start()
    cp_wo.start()
    proj(0, 1, kn)
    prep_w(2)
    cp_x2.wait()
    proj(0, 2, vn)
    ln0(T, S)
    cp_wo.wait()
    for c in cp_w1 + cp_w2:
        c.start()
    for j in range(NJ):
        wo[:, pl.ds(j * 128, 128)] = permute_rows(woraw[:, pl.ds(j * 128, 128)].astype(f32))
    jax.lax.fori_loop(0, 2, layer, None)
    for i in range(NB):
        pltpu.make_async_copy(xio.at[pl.ds(i * TB, TB)], out_hbm.at[pl.ds(i * TB, TB)], sem_out.at[i]).wait()


@jax.jit
def pallas_interleave_layers__sliding_local_dilated__mixer_token_mlp__prompt_kernel(
    A_x, A_wqkv, A_wo, B_x, B_w1, B_b1, B_w2, B_b2,
):
    del B_x
    any_spec = pl.BlockSpec(memory_space=pl.ANY)
    vmem_spec = pl.BlockSpec(memory_space=pltpu.VMEM)
    out = pl.pallas_call(
        _kernel,
        out_shape=jax.ShapeDtypeStruct((S, D), bf16),
        in_specs=[any_spec, any_spec, any_spec, any_spec, vmem_spec, any_spec, vmem_spec],
        out_specs=any_spec,
        scratch_shapes=[
            pltpu.VMEM((S, D), bf16),
            pltpu.VMEM((3, D, D), bf16),
            pltpu.VMEM((D, D), bf16),
            pltpu.VMEM((3, D, D), bf16),
            pltpu.VMEM((D, D), bf16),
            pltpu.VMEM((NF, S, FC), bf16),
            pltpu.VMEM((NB, F, TB), bf16),
            pltpu.VMEM((S, D), f32),
            pltpu.VMEM((S, D), bf16),
            pltpu.VMEM((D, S), bf16),
            pltpu.VMEM((D, F), bf16),
            pltpu.VMEM((NJ, T, 128), f32),
            pltpu.VMEM((NJ, T, 128), f32),
            pltpu.VMEM((NJ, T, 128), f32),
            pltpu.VMEM((NJ, T, 128), f32),
            pltpu.VMEM((NJ, T + HALO, 128), f32),
            pltpu.VMEM((NJ, T + HALO, 128), f32),
            pltpu.VMEM((T, D), bf16),
            pltpu.SemaphoreType.DMA((6,)),
            pltpu.SemaphoreType.DMA((NF,)),
            pltpu.SemaphoreType.DMA((NB,)),
            pltpu.SemaphoreType.DMA((NB,)),
        ],
        compiler_params=pltpu.CompilerParams(vmem_limit_bytes=110 * 1024 * 1024),
        name="interleave_layers",
    )(A_x.reshape(S, D), A_wqkv, A_wo, B_w1, B_b1, B_w2, B_b2)
    return out.reshape(1, S, D)
```
